```python
import os as _os
_os.environ.setdefault('JAX_PLATFORMS', 'cpu')
import jax
import jax.numpy as jnp

def _softmax(x, axis=-1):
    return jax.nn.softmax(x, axis=axis)

def _gelu(x):
    return jax.nn.gelu(x, approximate=True)

def _silu(x):
    return jax.nn.silu(x)

def _sigmoid(x):
    return jax.nn.sigmoid(x)

def _layernorm(x, axis=-1, eps=1e-05):
    m = jnp.mean(x, axis=axis, keepdims=True)
    v = jnp.var(x, axis=axis, keepdims=True)
    return (x - m) / jnp.sqrt(v + eps)

def _scatter_add(tgt, idx, src, axis=0):
    return tgt.at[idx].add(src)

def _segment_sum(src, seg, n):
    return jax.ops.segment_sum(src, seg, n)

class _Rng:

    def __init__(self, key):
        self._k = key

    def _next(self):
        self._k, sub = jax.random.split(self._k)
        return sub

    def normal(self, shape):
        return jax.random.normal(self._next(), shape, dtype=jnp.bfloat16)

    def randint(self, lo, hi, shape):
        return jax.random.randint(self._next(), shape, lo, hi, dtype=jnp.int32)

    def uniform(self, shape, lo=0.0, hi=1.0):
        return jax.random.uniform(self._next(), shape, jnp.bfloat16, lo, hi)

    def permutation(self, n):
        return jax.random.permutation(self._next(), n)
kernel_name = 'adaLN_cond__memory_aug_recurrent_mem_tr__moe_arch_mod__prompt'

def setup_inputs():
    _rng = _Rng(jax.random.key(int.from_bytes(__import__("os").urandom(4), "little")))
    _w = lambda a: (lambda t: t.astype(jnp.bfloat16) if jnp.issubdtype(t.dtype, jnp.floating) else t)(jnp.asarray(a))

    def _A_setup():
        B, S, Dm = (1, 2048, 448)
        H, Dh = (16, 256)
        M, seg = (8, 32)
        seg = min(seg, S)
        S = S // seg * seg
        return {'x': _w((lambda *s: _rng.normal(s) * 0.05)(B, S, Dm)), 'mem0': _w((lambda *s: _rng.normal(s) * 0.4)(B, M, Dm)), 'Wq': _w((lambda *s: _rng.normal(s) * 1.6)(Dm, H, Dh) * Dm ** (-0.5)), 'Wk': _w((lambda *s: _rng.normal(s) * 1.6)(Dm, H, Dh) * Dm ** (-0.5)), 'Wv': _w((lambda *s: _rng.normal(s) * 0.4)(Dm, H, Dh) * Dm ** (-0.5)), 'Wo': _w((lambda *s: _rng.normal(s) * 0.4)(H, Dh, Dm) * (H * Dh) ** (-0.5)), 'seg_len': seg}
    _A_in = _A_setup()

    def _B_setup():
        B, S, D, F, C = (1, 2048, 448, 1792, 1)
        return {'x': _w((lambda *s: _rng.normal(s) * 0.05)(B, S, D)), 'w_r': _w((lambda *s: _rng.normal(s) * 0.05)(D)), 'w_gate': _w((lambda *s: _rng.normal(s) * 0.05)(D, F)), 'w_up': _w((lambda *s: _rng.normal(s) * 0.05)(D, F)), 'w_down': _w((lambda *s: _rng.normal(s) * 0.05)(F, D))}
    _B_in = _B_setup()
    return {'A_x': _A_in['x'], 'A_mem0': _A_in['mem0'], 'A_Wq': _A_in['Wq'], 'A_Wk': _A_in['Wk'], 'A_Wv': _A_in['Wv'], 'A_Wo': _A_in['Wo'], 'A_seg_len': _A_in['seg_len'], 'B_x': _B_in['x'], 'B_w_r': _B_in['w_r'], 'B_w_gate': _B_in['w_gate'], 'B_w_up': _B_in['w_up'], 'B_w_down': _B_in['w_down'], 'c': _w((lambda *s: _rng.normal(s) * 0.05)(1, 448) * 8.0), 'w_mod': _w((lambda *s: _rng.normal(s) * 0.05)(448, 6 * 448) * 448 ** (-0.5) * 8.0)}

def reference(A_x, A_mem0, A_Wq, A_Wk, A_Wv, A_Wo, A_seg_len, B_x, B_w_r, B_w_gate, B_w_up, B_w_down, c, w_mod):

    def _A_ref(x, mem0, Wq, Wk, Wv, Wo, seg_len):
        B, S, Dm = x.shape
        H, Dh = (Wq.shape[1], Wq.shape[2])
        M = mem0.shape[1]
        scale = Dh ** (-0.5)
        n_seg = S // seg_len
        L = M + seg_len
        idx = jnp.arange(L)
        mask = (idx[:, None] < M) | (idx[:, None] >= idx[None, :])
        mem = mem0
        outs = []
        for s in range(n_seg):
            xs = x[:, s * seg_len:(s + 1) * seg_len, :].copy()
            h = jnp.concatenate([mem, xs], axis=1)
            q = jnp.einsum('btd,dhe->bhte', h, Wq)
            k = jnp.einsum('btd,dhe->bhte', h, Wk)
            v = jnp.einsum('btd,dhe->bhte', h, Wv)
            scores = jnp.einsum('bhqe,bhke->bhqk', q, k) * scale
            scores = jnp.where(mask[None, None], scores, -1000000000.0)
            p = _softmax(scores, axis=-1)
            o = jnp.einsum('bhqk,bhke->bhqe', p, v)
            o = jnp.einsum('bhte,hed->btd', o, Wo)
            mem = o[:, :M, :].copy()
            outs.append(o[:, M:, :])
        return jnp.concatenate(outs, axis=1)

    def _B_ref(x, w_r, w_gate, w_up, w_down):
        B, S, D = x.shape
        C = 1
        r = x @ w_r
        idx = jnp.argsort(-r, axis=-1)[:, :C]
        idx_e = jnp.repeat(idx.reshape(B, C, 1), D, axis=2)
        x_sel = jnp.take_along_axis(x, idx_e, axis=1)
        g = _silu(x_sel @ w_gate)
        u = x_sel @ w_up
        y = g * u @ w_down
        r_sel = _sigmoid(jnp.take_along_axis(r, idx, axis=1))
        y = y * r_sel.reshape(B, C, 1)
        b_off = (jnp.arange(B) * S).reshape(B, 1)
        flat_idx = (idx + b_off).reshape(B * C)
        zero = (x * 0.0).reshape(B * S, D)
        upd = _scatter_add(zero, flat_idx, y.reshape(B * C, D), axis=0)
        return x + upd.reshape(B, S, D)
    x = A_x
    mod = (_silu(c) @ w_mod).reshape(c.shape[0], 6, 1, -1)
    sa, ca, ga, sb, cb, gb = (mod[:, 0].copy(), mod[:, 1].copy(), mod[:, 2].copy(), mod[:, 3].copy(), mod[:, 4].copy(), mod[:, 5].copy())
    h = _layernorm(x, axis=-1) * (1 + ca) + sa
    x = x + ga * _A_ref(h, A_mem0, A_Wq, A_Wk, A_Wv, A_Wo, A_seg_len)
    h = _layernorm(x, axis=-1) * (1 + cb) + sb
    x = x + gb * _B_ref(h, B_w_r, B_w_gate, B_w_up, B_w_down)
    return x
```

```python
import functools

import jax
import jax.numpy as jnp
from jax import lax
import jax.experimental.pallas as pl
import jax.experimental.pallas.tpu as pltpu

F32 = jnp.float32
BF16 = jnp.bfloat16
U32 = jnp.uint32

D = 448
DP = 512
H = 16
DH = 256
M = 8
SEG = 32
L = SEG + M
BLK = 128
NG = 28
KV = L * 8
EPS = 1e-5
HALVES = ((0, D // 2), (D // 2, D))
AHEAD = 3


def _r16(x):
    return x.astype(BF16).astype(F32)


def _dot(a, b):
    return lax.dot_general(a, b, (((1,), (0,)), ((), ())), preferred_element_type=F32)


def _dot_nt(a, b):
    return lax.dot_general(a, b, (((1,), (1,)), ((), ())), preferred_element_type=F32)


def _pack2(a, b):
    return pltpu.pack_elementwise([a, b], packed_dtype=BF16)


def _words(x):
    return pltpu.bitcast(x.astype(BF16), U32)


def _unwords(w):
    return pltpu.bitcast(w, BF16)


def _repeat_tail(x, axis):
    tail = lax.slice_in_dim(x, D - 64, D, axis=axis)
    return jnp.concatenate([x, tail], axis=axis)


def _row_sum(x):
    left = lax.broadcasted_iota(jnp.int32, (x.shape[0], 128), 1) < 64
    t = (x[:, 0:128] + x[:, 128:256]) + (x[:, 256:384] + jnp.where(left, x[:, 384:512], 0.0))
    return jnp.sum(t, axis=1, keepdims=True)


def _ln_mod(x, scale1, shift):
    xc = x - _row_sum(x) / D
    var = _row_sum(xc * xc) / D
    den = _r16(jnp.sqrt(_r16(_r16(var) + _r16(jnp.float32(EPS)))))
    return ((xc / den) * scale1 + shift).astype(BF16)


def _kernel(x_hbm, mem0_hbm, wq_hbm, wk_hbm, wv_hbm, wo_hbm, wr_hbm, wg_hbm, wu_hbm,
            wd_hbm, c_hbm, wmod_hbm, out_hbm, c_v, mem0_v, wr_v,
            x_v, wq_v, wk_v, wv_v, wo_v, wg_v, wu_v, wd_v, wmod_v,
            qh_s, w1_s, w2_s, wc_s, k0_s, k1_s, k2_s, k3_s, v0_s, v1_s, v2_s, v3_s, xs, o_s, x1_s, y_s, out_v, vec_s, sems, osem,
            *, n_blk, gchunk, first, lead, dup, xlu_t, iters, nstep, K_CHUNKS, funroll, bunroll):
    kw_s = (k0_s, k1_s, k2_s, k3_s)
    vw_s = (v0_s, v1_s, v2_s, v3_s)

    queue = []

    def fetch(src, dst):
        queue.append(pltpu.make_async_copy(src, dst, sems.at[len(queue)]))
        return len(queue) - 1

    def fetch_rows(src, dst, r0, r1):
        return [fetch(src.at[pl.ds(r0 * H, (r1 - r0) * H), pl.ds(128 * j, 128)],
                      dst.at[j, pl.ds(r0 * H // 2, (r1 - r0) * H // 2), :].bitcast(BF16))
                for j in range(2)]

    cp_q = [fetch_rows(wq_hbm, wq_v, r0, r1) for r0, r1 in HALVES]
    cp_k = [fetch_rows(wk_hbm, wk_v, r0, r1) for r0, r1 in K_CHUNKS]
    cp_v = [fetch_rows(wv_hbm, wv_v, r0, r1) for r0, r1 in HALVES]
    o_first = len(queue)
    for t in range(H // 4):
        fetch(wo_hbm.at[pl.ds(4 * D * t, 4 * D), :], wo_v.at[pl.ds(4 * D * t, 4 * D), :])
    cp_small = [fetch(c_hbm, c_v), fetch(mem0_hbm, mem0_v), fetch(wr_hbm, wr_v)]
    cp_mod = fetch(wmod_hbm, wmod_v)
    cp_x = [fetch(x_hbm.at[:, pl.ds(BLK * b, BLK)], x_v.at[b].bitcast(BF16)) for b in range(n_blk)]
    cp_ffn = [fetch(wg_hbm, wg_v), fetch(wu_hbm, wu_v), fetch(wd_hbm, wd_v)]
    issued = [0]

    def issue(upto):
        while issued[0] < min(upto, len(queue)):
            queue[issued[0]].start()
            issued[0] += 1

    def arrive(cps, ahead=AHEAD):
        for cp in cps:
            issue(cp + ahead + 1)
            queue[cp].wait()

    SA, CA, GA, SB, CB, GB, WR = range(7)

    def modulation():
        cf = jnp.broadcast_to(c_v[...].astype(F32), (8, D))
        sc = _r16(cf * jax.nn.sigmoid(cf))
        mod = _r16(_dot(sc, wmod_v[...]))
        for i in range(6):
            v = mod[:, D * i:D * (i + 1)]
            vec_s[i] = _repeat_tail(_r16(1.0 + v) if i in (CA, CB) else v, 1)
        wr = jnp.broadcast_to(wr_v[...].astype(F32).reshape(1, D), (8, D))
        vec_s[WR] = _repeat_tail(wr, 1)

    def vec(i, rows):
        return jnp.concatenate([vec_s[i]] * (rows // 8), axis=0)

    def lanes(b):
        return pl.ds(pl.multiple_of(b * BLK, BLK), BLK)

    def seg_rows(i):
        return slice(SEG // 2 * i, SEG // 2 * (i + 1))

    def load_tokens(b):
        xs[b] = pltpu.bitcast(_repeat_tail(_unwords(x_v[b]), 0).T, U32)

    def norm_segment(b, i):
        x = _unwords(xs[b, seg_rows(i), :]).astype(F32)
        return _ln_mod(x, vec(CA, SEG), vec(SA, SEG))

    def store_tokens(b):
        out_v[b] = pltpu.bitcast(_unwords(y_s[b]).T[0:D], U32)

    def out_copy(b):
        return pltpu.make_async_copy(out_v.at[b].bitcast(BF16), out_hbm.at[:, lanes(b)], osem)

    def head_pair(w_v, s, r0=0, r1=D):
        words = jnp.concatenate(
            [w_v[j, pl.ds(r0 * 8 + s, r1 - r0, stride=8), :] for j in range(2)], axis=1)
        lo = pltpu.bitcast(words << 16, F32)
        hi = pltpu.bitcast(words & jnp.uint32(0xFFFF0000), F32)
        return lo, hi

    def store_group(g, xw, yw, r0, r1):
        if r0 == 0:
            y1 = _r16(yw[0:64])
            w1_s[g, 0:32, :] = _words(xw[0:64] - y1)
            wc_s[g, 0:32, :] = _words(y1)
        lo, hi = max(r0, 64), min(r1, 384)
        if lo < hi:
            w1_s[g, lo // 2:hi // 2, :] = _words(xw[lo - r0:hi - r0])
            w2_s[g, lo // 2:hi // 2, :] = _words(yw[lo - r0:hi - r0])
        if r1 == D:
            x7 = _r16(xw[384 - r0:])
            w2_s[g, 0:32, :] = _words(yw[384 - r0:] - x7)
            wc_s[g, 32:64, :] = _words(x7)

    def fold(base, lhs_v, rhs_rows, scale, r0, r1, before=None):
        left = lax.broadcasted_iota(jnp.int32, (r1 - r0, 128), 1) < 64

        def body(t, carry):
            if before is not None:
                before(t)
            shared = []
            for i in range(2):
                s = 2 * t + i
                la, lb = head_pair(lhs_v, s, r0, r1)
                ra, rb = rhs_rows(s)
                pa = _dot_nt(la, ra[0:384])
                pb = _dot_nt(lb, rb[0:384])
                pad = -(r1 - r0) % 128
                tails = []
                for lhs, rhs in ((la, ra), (lb, rb)):
                    lhs = lhs.astype(BF16)
                    if pad:
                        lhs = jnp.concatenate([lhs, lhs[0:pad]], axis=0)
                    tails.append(_dot_nt(rhs[384:448], lhs))
                tail = jnp.concatenate(tails, axis=0).T[0:r1 - r0]
                if scale is not None:
                    pa, pb, tail = pa * scale, pb * scale, tail * scale
                for j in range(3):
                    store_group(base + 8 * j + s, pa[:, 128 * j:128 * (j + 1)],
                                pb[:, 128 * j:128 * (j + 1)], r0, r1)
                shared.append(tail)
            store_group(base + 24 + t, shared[0], shared[1], r0, r1)
            return carry
        lax.fori_loop(0, H // 4, body, 0, unroll=funroll)

    def split_q_heads(r0, r1):
        def body(s, carry):
            for i, q in enumerate(head_pair(wq_v, s, r0, r1)):
                qh_s[2 * s + i, r0 // 2:r1 // 2, :] = _words(q)
            return carry
        lax.fori_loop(0, H // 2, body, 0)

    def q_rows(s):
        return _unwords(qh_s[2 * s]), _unwords(qh_s[2 * s + 1])

    def o_rows(s):
        r0 = pl.multiple_of(s * 2 * D, 2 * D)
        return wo_v[pl.ds(r0, D), :], wo_v[pl.ds(r0 + D, D), :]

    def o_arrive(t):
        rows = pl.ds(pl.multiple_of(t * 4 * D, 4 * D), 4 * D)
        pltpu.make_async_copy(wo_hbm.at[rows, :], wo_v.at[rows, :], sems.at[o_first + t]).wait()

    with jax.named_scope("wait_q"):
        for cps, (r0, r1) in zip(cp_q, HALVES):
            arrive(cps)
            split_q_heads(r0, r1)
    for cps, (r0, r1) in zip(cp_k, K_CHUNKS):
        with jax.named_scope(f"wait_k{r0}"):
            arrive(cps)
            if r1 == D:
                issue(o_first + H // 4)
        with jax.named_scope(f"fold_a{r0}"):
            fold(0, wk_v, q_rows, DH ** -0.5, r0, r1)
    with jax.named_scope("wait_v"):
        for cps in cp_v:
            arrive(cps)
        issue(len(queue))
    with jax.named_scope("fold_b"):
        fold(NG, wv_v, o_rows, None, 0, D, o_arrive)
    with jax.named_scope("wait_mod"):
        arrive(cp_small + [cp_mod])
    with jax.named_scope("mod"):
        modulation()
    arrive(cp_x)
    load_tokens(0)
    load_tokens(min(1, n_blk - 1))
    y_s[n_blk, seg_rows(0), :] = pltpu.bitcast(norm_segment(0, 0), U32)
    o_s[...] = jnp.zeros(o_s.shape, F32)

    left_l = lax.broadcasted_iota(jnp.int32, (L, 128), 1) < 64
    half_mask = jnp.where(left_l, jnp.uint32(0x0000FFFF), jnp.uint32(0xFFFF0000))
    causal = (lax.broadcasted_iota(jnp.int32, (8, 128), 1) // H
              <= lax.broadcasted_iota(jnp.int32, (8, 128), 0))

    def wt(ref, g, rows=slice(None)):
        return pltpu.bitcast(ref[g, rows, :], BF16)

    def emit(g, a, b):
        dst = vw_s if g >= NG else kw_s
        t = g % NG
        if t < 24:
            dst[t // 8][pl.ds(t % 8, L, stride=8), :] = _pack2(a, b)
        else:
            for i, v in enumerate((a, b)):
                w = _pack2(v, v) & half_mask
                if dup and g >= NG:
                    w = w | pltpu.roll(w, 64, 1)
                dst[3][pl.ds(2 * (t - 24) + i, L, stride=8), :] = w

    def project(groups, lhs1, lhs2, lhsc):
        def w(ref):
            return jnp.concatenate([wt(ref, g) for g in groups], axis=1)
        c = _dot(lhsc, w(wc_s))
        o1 = _dot(lhs1, w(w1_s)) + c
        o2 = _dot(lhs2, w(w2_s)) + c
        for i, g in enumerate(groups):
            emit(g, o1[:, 128 * i:128 * (i + 1)], o2[:, 128 * i:128 * (i + 1)])

    def project_by_k(groups, lhs1, lhs2, lhsc):
        def w(ref, k):
            return jnp.concatenate([wt(ref, g, slice(64 * k, 64 * (k + 1))) for g in groups],
                                   axis=1)
        c = _dot(lhsc, w(wc_s, 0))
        o1, o2 = c, c
        for k in range(3):
            o1 = o1 + _dot(lhs1[:, 128 * k:128 * (k + 1)], w(w1_s, k))
            o2 = o2 + _dot(lhs2[:, 128 * k:128 * (k + 1)], w(w2_s, k))
        for i, g in enumerate(groups):
            emit(g, o1[:, 128 * i:128 * (i + 1)], o2[:, 128 * i:128 * (i + 1)])

    def all_keys(v, op):
        v = op(v, pltpu.roll(v, 64, 1))
        v = op(v, pltpu.roll(v, 32, 1))
        return op(v, pltpu.roll(v, 16, 1))

    def chunks(gs):
        return [gs[i:i + gchunk] for i in range(0, len(gs), gchunk)]

    def finish_segment(b, i, valid, best):
        x1 = (_unwords(xs[b, seg_rows(i), :]).astype(F32)
              + _r16(vec(GA, SEG) * o_s[...])).astype(BF16)
        x1_s[b, seg_rows(i), :] = pltpu.bitcast(x1, U32)
        x1 = x1.astype(F32)
        h2 = _ln_mod(x1, vec(CB, SEG), vec(SB, SEG)).astype(F32)
        r = _r16(_row_sum(h2 * vec(WR, SEG)))
        y_s[b, seg_rows(i), :] = _words(x1 + vec(GB, SEG) * (h2 + h2 * 0.0))
        better = r > best[0]
        if valid is not None:
            better = better & valid
        idx = b * BLK + SEG * i + lax.broadcasted_iota(jnp.int32, (SEG, 1), 0)
        return jnp.where(better, r, best[0]), jnp.where(better, idx, best[1])

    def step(b, i, carry):
        mem, best = carry
        z = jnp.concatenate([_unwords(y_s[n_blk, seg_rows(0), :]).astype(F32), mem], axis=0)
        if i:
            best = finish_segment(b, i - 1, None, best)
        else:
            valid = jnp.broadcast_to(b, (SEG, 1)) > 0
            best = finish_segment(jnp.maximum(b - 1, 0), BLK // SEG - 1, valid, best)
        if i + 1 < BLK // SEG:
            nxt = norm_segment(b, i + 1)
        else:
            nxt = norm_segment(jnp.minimum(b + 1, n_blk - 1), 0)
        y_s[n_blk, seg_rows(0), :] = pltpu.bitcast(nxt, U32)
        z0, zd = z[:, 0:128], z[:, 384:512]
        lhs1 = z[:, 0:384]
        lhs2 = jnp.concatenate([jnp.where(left_l, zd, z0), z[:, 128:384]], axis=1)
        lhsc = jnp.where(left_l, z0, zd)

        order = list(range(24, 28)) + list(range(24))
        keys = {}

        def keys_done(g):
            j = {27: 3, 7: 0, 15: 1, 23: 2}.get(g)
            if j is not None:
                k = pltpu.bitcast(kw_s[j][...], BF16)
                keys[j] = k.T

        if first:
            project_by_k(order[:first], lhs1, lhs2, lhsc)
            keys_done(order[first - 1])
        for gs in chunks(order[first:]):
            project(gs, lhs1, lhs2, lhsc)
            keys_done(gs[-1])
        vb = [NG + g for g in order]
        for gs in chunks(vb[:lead]):
            project(gs, lhs1, lhs2, lhsc)
        tiles = []
        for n in range(L // 8):
            q0 = 8 * n if 8 * n < SEG else 0
            kt = jnp.concatenate([keys[j][:, 128 * n:128 * (n + 1)] for j in range(4)], axis=0)
            t = _dot(z[q0:L], kt)
            if 8 * n < SEG:
                t = jnp.concatenate([jnp.where(causal, t[0:8], -1e9), t[8:]], axis=0)
            if q0:
                t = jnp.concatenate([jnp.full((q0, 128), -1e9, F32), t], axis=0)
            tiles.append(t)
        mx = all_keys(functools.reduce(jnp.maximum, tiles), jnp.maximum)
        ex = [jnp.exp(t - mx) for t in tiles]
        inv = 1.0 / all_keys(functools.reduce(jnp.add, ex), jnp.add)
        p = _r16(jnp.concatenate([e * inv for e in ex], axis=1))
        for gs in chunks(vb[lead:]):
            project(gs, lhs1, lhs2, lhsc)

        o = _dot(p, jnp.concatenate([pltpu.bitcast(vw_s[j][...], BF16) for j in (3, 0, 1, 2)], axis=1))
        o3 = o[:, 0:128]
        if not dup:
            o3 = o3 + pltpu.roll(o3, 64, 1)
        o = _r16(jnp.concatenate([o[:, 128:512], o3], axis=1))

        o_s[...] = o[0:SEG]
        return o[SEG:L], best

    def block(b, carry):
        for i in range(nstep or BLK // SEG):
            carry = step(b, i, carry)
        load_tokens(jnp.minimum(b + 2, n_blk - 1))
        store_tokens(jnp.maximum(b - 1, 0))

        @pl.when(b > 0)
        def _():
            out_copy(b - 1).start()
        return carry

    mem = _repeat_tail(mem0_v[...].astype(F32), 1)
    best = (jnp.full((SEG, 1), -jnp.inf, F32), lax.broadcasted_iota(jnp.int32, (SEG, 1), 0))
    with jax.named_scope("main"):
      _, best = lax.fori_loop(0, iters or n_blk, block, (mem, best), unroll=bunroll)
    best_r, best_i = finish_segment(n_blk - 1, BLK // SEG - 1, None, best)
    store_tokens(n_blk - 1)
    out_copy(n_blk - 1).start()

    top = jnp.max(best_r)
    idx = jnp.min(jnp.where(best_r == top, best_i, n_blk * BLK - 1))
    sel_b = idx // BLK
    sel_r = pl.ds(pl.multiple_of(((idx - sel_b * BLK) // 16) * 8, 8), 8)
    x1 = _unwords(x1_s[sel_b, sel_r, :]).astype(F32)
    h2 = _ln_mod(x1, vec(CB, 16), vec(SB, 16)).astype(F32)
    r = _r16(_row_sum(h2 * vec(WR, 16)))
    arrive(cp_ffn)
    g = _r16(_dot(h2[:, 0:D], wg_v[...]))
    g = _r16(g * jax.nn.sigmoid(g))
    u = _r16(_dot(h2[:, 0:D], wu_v[...]))
    y = _r16(_dot_nt(_r16(g * u), _repeat_tail(wd_v[...], 0)))
    y = _r16(y * _r16(jax.nn.sigmoid(r)))
    hit = (lax.broadcasted_iota(jnp.int32, (16, 1), 0) == idx % 16)
    upd = h2 * 0.0 + jnp.where(hit, y, 0.0)
    y_s[sel_b, sel_r, :] = _words(x1 + vec(GB, 16) * _r16(h2 + upd))
    for b in range(iters or n_blk):
        out_copy(b).wait()
    store_tokens(sel_b)
    last = out_copy(sel_b)
    last.start()
    last.wait()


def _make(gchunk=1, first=4, lead=10, dup=True, xlu_t=True, flags=None, iters=0, nstep=0, kc=((0, 128), (128, D)), funroll=2, bunroll=1):
    def fn(A_x, A_mem0, A_Wq, A_Wk, A_Wv, A_Wo, A_seg_len, B_x, B_w_r, B_w_gate, B_w_up,
           B_w_down, c, w_mod):
        del A_seg_len, B_x
        _, S, _ = A_x.shape
        F = B_w_gate.shape[1]
        n_blk = S // BLK
        hbm = pl.BlockSpec(memory_space=pltpu.HBM)
        vmem = pl.BlockSpec(memory_space=pltpu.VMEM)
        out_t = pl.pallas_call(
            functools.partial(_kernel, n_blk=n_blk, gchunk=gchunk, first=first, lead=lead,
                              dup=dup, xlu_t=xlu_t, iters=iters, nstep=nstep, K_CHUNKS=kc, funroll=funroll, bunroll=bunroll),
            out_shape=jax.ShapeDtypeStruct((D, S), BF16),
            in_specs=[hbm] * 12,
            out_specs=hbm,
            scratch_shapes=[
                pltpu.VMEM((1, D), BF16),
                pltpu.VMEM((M, D), BF16),
                pltpu.VMEM((D,), BF16),
                pltpu.VMEM((n_blk, D // 2, BLK), U32),
                pltpu.VMEM((2, D * H // 2, 128), U32),
                pltpu.VMEM((2, D * H // 2, 128), U32),
                pltpu.VMEM((2, D * H // 2, 128), U32),
                pltpu.VMEM((H * D, DH), BF16),
                pltpu.VMEM((D, F), BF16),
                pltpu.VMEM((D, F), BF16),
                pltpu.VMEM((D, F), BF16),
                pltpu.VMEM((D, 6 * D), BF16),
                pltpu.VMEM((H, D // 2, DH), U32),
                pltpu.VMEM((2 * NG, 192, 128), U32),
                pltpu.VMEM((2 * NG, 192, 128), U32),
                pltpu.VMEM((2 * NG, 64, 128), U32),
                *[pltpu.VMEM((KV, 128), U32)] * 8,
                pltpu.VMEM((n_blk, BLK // 2, DP), U32),
                pltpu.VMEM((SEG, DP), F32),
                pltpu.VMEM((n_blk, BLK // 2, DP), U32),
                pltpu.VMEM((n_blk + 1, BLK // 2, DP), U32),
                pltpu.VMEM((n_blk, D // 2, BLK), U32),
                pltpu.VMEM((7, 8, DP), F32),
                pltpu.SemaphoreType.DMA((48,)),
                pltpu.SemaphoreType.DMA(()),
            ],
            compiler_params=pltpu.CompilerParams(vmem_limit_bytes=100 * 1024 * 1024, flags=flags),
        )(A_x.reshape(S, D).T, A_mem0.reshape(M, D), A_Wq.reshape(D * H, DH),
          A_Wk.reshape(D * H, DH), A_Wv.reshape(D * H, DH),
          A_Wo.transpose(0, 2, 1).reshape(H * D, DH),
          B_w_r, B_w_gate, B_w_up, B_w_down.T, c, w_mod)
        return out_t.T.reshape(A_x.shape)
    return fn


@jax.jit
def pallas_adaLN_cond__memory_aug_recurrent_mem_tr__moe_arch_mod__prompt_kernel(
        A_x, A_mem0, A_Wq, A_Wk, A_Wv, A_Wo, A_seg_len, B_x, B_w_r, B_w_gate, B_w_up, B_w_down,
        c, w_mod):
    return _make()(A_x, A_mem0, A_Wq, A_Wk, A_Wv, A_Wo, A_seg_len, B_x, B_w_r, B_w_gate, B_w_up,
                   B_w_down, c, w_mod)
```

```python
import functools

import jax
import jax.numpy as jnp
from jax import lax
import jax.experimental.pallas as pl
import jax.experimental.pallas.tpu as pltpu

F32 = jnp.float32
BF16 = jnp.bfloat16
U32 = jnp.uint32

D = 448
DP = 512
H = 16
DH = 256
M = 8
SEG = 32
L = SEG + M
BLK = 128
NG = 28
EPS = 1e-5
MASKED = -1e9

HALVES = ((0, D // 2), (D // 2, D))
K_CHUNKS = ((0, 128), (128, D))
AHEAD = 3
CHUNK = 4
LEAD = 8


def _r16(x):
    return x.astype(BF16).astype(F32)


def _dot(a, b):
    return lax.dot_general(a, b, (((1,), (0,)), ((), ())), preferred_element_type=F32)


def _dot_nt(a, b):
    return lax.dot_general(a, b, (((1,), (1,)), ((), ())), preferred_element_type=F32)


def _words(x):
    return pltpu.bitcast(x.astype(BF16), U32)


def _unwords(w):
    return pltpu.bitcast(w, BF16)


def _pack2(a, b):
    return (pltpu.bitcast(_r16(a), U32) >> 16) | pltpu.bitcast(_r16(b), U32)


def _repeat_tail(x, axis):
    return jnp.concatenate([x, lax.slice_in_dim(x, D - 64, D, axis=axis)], axis=axis)


def _row_sum(x):
    left = lax.broadcasted_iota(jnp.int32, (x.shape[0], 128), 1) < 64
    t = (x[:, 0:128] + x[:, 128:256]) + (x[:, 256:384] + jnp.where(left, x[:, 384:512], 0.0))
    return jnp.sum(t, axis=1, keepdims=True)


def _ln_mod(x, scale1, shift):
    xc = x - _row_sum(x) / D
    var = _row_sum(xc * xc) / D
    den = _r16(jnp.sqrt(_r16(_r16(var) + _r16(jnp.float32(EPS)))))
    return ((xc / den) * scale1 + shift).astype(BF16)


def _kernel(x_hbm, mem0_hbm, wq_hbm, wk_hbm, wv_hbm, wo_hbm, wr_hbm, wg_hbm, wu_hbm, wd_hbm,
            c_hbm, wmod_hbm, out_hbm,
            c_v, mem0_v, wr_v, x_v, wq_v, wk_v, wv_v, wo_v, wg_v, wu_v, wd_v, wmod_v,
            qh_s, w1_s, w2_s, wc_s, k0_s, k1_s, k2_s, k3_s, v0_s, v1_s, v2_s, v3_s,
            xs_s, o_s, x1_s, y_s, out_v, vec_s, sems, out_sem, *, n_blk):
    k_s = (k0_s, k1_s, k2_s, k3_s)
    v_s = (v0_s, v1_s, v2_s, v3_s)

    queue = []
    issued = [0]

    def fetch(src, dst):
        queue.append(pltpu.make_async_copy(src, dst, sems.at[len(queue)]))
        return len(queue) - 1

    def fetch_rows(src, dst, r0, r1):
        return [fetch(src.at[pl.ds(r0 * H, (r1 - r0) * H), pl.ds(128 * j, 128)],
                      dst.at[j, pl.ds(r0 * H // 2, (r1 - r0) * H // 2), :].bitcast(BF16))
                for j in range(2)]

    def issue(upto):
        while issued[0] < min(upto, len(queue)):
            queue[issued[0]].start()
            issued[0] += 1

    def arrive(copies):
        for i in copies:
            issue(i + AHEAD + 1)
            queue[i].wait()

    cp_q = [fetch_rows(wq_hbm, wq_v, r0, r1) for r0, r1 in HALVES]
    cp_k = [fetch_rows(wk_hbm, wk_v, r0, r1) for r0, r1 in K_CHUNKS]
    cp_v = [fetch_rows(wv_hbm, wv_v, r0, r1) for r0, r1 in HALVES]
    cp_o = [fetch(wo_hbm.at[pl.ds(4 * D * t, 4 * D), :], wo_v.at[pl.ds(4 * D * t, 4 * D), :])
            for t in range(H // 4)]
    cp_small = [fetch(c_hbm, c_v), fetch(mem0_hbm, mem0_v), fetch(wr_hbm, wr_v),
                fetch(wmod_hbm, wmod_v)]
    cp_x = [fetch(x_hbm.at[:, pl.ds(BLK * b, BLK)], x_v.at[b].bitcast(BF16))
            for b in range(n_blk)]
    cp_ffn = [fetch(wg_hbm, wg_v), fetch(wu_hbm, wu_v), fetch(wd_hbm, wd_v)]

    def head_pair(w_v, s, r0, r1):
        words = jnp.concatenate(
            [w_v[j, pl.ds(r0 * 8 + s, r1 - r0, stride=8), :] for j in range(2)], axis=1)
        return (pltpu.bitcast(words << 16, F32),
                pltpu.bitcast(words & jnp.uint32(0xFFFF0000), F32))

    def store_group(g, xw, yw, r0, r1):
        if r0 == 0:
            y1 = _r16(yw[0:64])
            w1_s[g, 0:32, :] = _words(xw[0:64] - y1)
            wc_s[g, 0:32, :] = _words(y1)
        lo, hi = max(r0, 64), min(r1, 384)
        w1_s[g, lo // 2:hi // 2, :] = _words(xw[lo - r0:hi - r0])
        w2_s[g, lo // 2:hi // 2, :] = _words(yw[lo - r0:hi - r0])
        if r1 == D:
            x7 = _r16(xw[384 - r0:])
            w2_s[g, 0:32, :] = _words(yw[384 - r0:] - x7)
            wc_s[g, 32:64, :] = _words(x7)

    def fold(base, lhs_v, rhs_pair, scale, r0, r1, before=None):
        def body(t, carry):
            if before is not None:
                before(t)
            tails = []
            for i in range(2):
                s = 2 * t + i
                la, lb = head_pair(lhs_v, s, r0, r1)
                ra, rb = rhs_pair(s)
                pa = _dot_nt(la, ra[0:384])
                pad = -(r1 - r0) % 128
                parts = []
                for lhs, rhs in ((la, ra), (lb, rb)):
                    lhs = lhs.astype(BF16)
                    if pad:
                        lhs = jnp.concatenate([lhs, lhs[0:pad]], axis=0)
                    parts.append(_dot_nt(rhs[384:D], lhs))
                tail = jnp.concatenate(parts, axis=0).T[0:r1 - r0]
                pb = _dot_nt(lb, rb[0:384])
                if scale is not None:
                    pa, pb, tail = pa * scale, pb * scale, tail * scale
                tails.append(tail)
                if i:
                    store_group(base + 24 + t, tails[0], tails[1], r0, r1)
                for j in range(3):
                    store_group(base + 8 * j + s, pa[:, 128 * j:128 * (j + 1)],
                                pb[:, 128 * j:128 * (j + 1)], r0, r1)
            return carry
        lax.fori_loop(0, H // 4, body, 0, unroll=2)

    def split_q_heads(r0, r1):
        def body(s, carry):
            for i, q in enumerate(head_pair(wq_v, s, r0, r1)):
                qh_s[2 * s + i, r0 // 2:r1 // 2, :] = _words(q)
            return carry
        lax.fori_loop(0, H // 2, body, 0)

    def q_pair(s):
        return _unwords(qh_s[2 * s]), _unwords(qh_s[2 * s + 1])

    def o_pair(s):
        r0 = pl.multiple_of(s * 2 * D, 2 * D)
        return wo_v[pl.ds(r0, D), :], wo_v[pl.ds(r0 + D, D), :]

    def o_arrive(t):
        rows = pl.ds(pl.multiple_of(t * 4 * D, 4 * D), 4 * D)
        pltpu.make_async_copy(wo_hbm.at[rows, :], wo_v.at[rows, :], sems.at[cp_o[0] + t]).wait()

    for copies, (r0, r1) in zip(cp_q, HALVES):
        arrive(copies)
        split_q_heads(r0, r1)
    for copies, (r0, r1) in zip(cp_k, K_CHUNKS):
        arrive(copies)
        if r1 == D:
            issue(cp_o[-1] + 1)
        fold(0, wk_v, q_pair, DH ** -0.5, r0, r1)
    for copies in cp_v:
        arrive(copies)
    issue(len(queue))
    fold(NG, wv_v, o_pair, None, 0, D, o_arrive)

    SA, CA, GA, SB, CB, GB, WR = range(7)

    def vec(i, rows):
        return jnp.concatenate([vec_s[i]] * (rows // 8), axis=0)

    def seg_rows(i):
        return slice(SEG // 2 * i, SEG // 2 * (i + 1))

    def load_tokens(b):
        xs_s[b] = pltpu.bitcast(_repeat_tail(_unwords(x_v[b]), 0).T, U32)

    def store_tokens(b):
        out_v[b] = pltpu.bitcast(_unwords(y_s[b]).T[0:D], U32)

    def out_copy(b):
        lanes = pl.ds(pl.multiple_of(b * BLK, BLK), BLK)
        return pltpu.make_async_copy(out_v.at[b].bitcast(BF16), out_hbm.at[:, lanes], out_sem)

    def norm_segment(b, i):
        x = _unwords(xs_s[b, seg_rows(i), :]).astype(F32)
        y_s[n_blk, seg_rows(0), :] = pltpu.bitcast(_ln_mod(x, vec(CA, SEG), vec(SA, SEG)), U32)

    def finish_segment(b, i, valid, best):
        x1 = (_unwords(xs_s[b, seg_rows(i), :]).astype(F32)
              + _r16(vec(GA, SEG) * o_s[...])).astype(BF16)
        x1_s[b, seg_rows(i), :] = pltpu.bitcast(x1, U32)
        x1 = x1.astype(F32)
        h2 = _ln_mod(x1, vec(CB, SEG), vec(SB, SEG)).astype(F32)
        r = _r16(_row_sum(h2 * vec(WR, SEG)))
        y_s[b, seg_rows(i), :] = _words(x1 + vec(GB, SEG) * (h2 + h2 * 0.0))
        better = r > best[0]
        if valid is not None:
            better = better & valid
        idx = b * BLK + SEG * i + lax.broadcasted_iota(jnp.int32, (SEG, 1), 0)
        return jnp.where(better, r, best[0]), jnp.where(better, idx, best[1])

    arrive(cp_small + cp_x)
    load_tokens(0)
    load_tokens(min(1, n_blk - 1))
    cf = jnp.broadcast_to(c_v[...].astype(F32), (8, D))
    mod = _r16(_dot(_r16(cf * jax.nn.sigmoid(cf)), wmod_v[...]))
    for i in range(6):
        v = mod[:, D * i:D * (i + 1)]
        vec_s[i] = _repeat_tail(_r16(1.0 + v) if i in (CA, CB) else v, 1)
    vec_s[WR] = _repeat_tail(jnp.broadcast_to(wr_v[...].astype(F32).reshape(1, D), (8, D)), 1)
    norm_segment(0, 0)
    o_s[...] = jnp.zeros(o_s.shape, F32)

    lane = lax.broadcasted_iota(jnp.int32, (L, 128), 1)
    left = lane < 64
    half_mask = jnp.where(left, jnp.uint32(0x0000FFFF), jnp.uint32(0xFFFF0000))
    causal = ((lax.broadcasted_iota(jnp.int32, (8, 128), 1) % 16) // 2
              <= lax.broadcasted_iota(jnp.int32, (8, 128), 0))

    def put(ref, s, words):
        ref[:, 8 * s:8 * (s + 1), :] = words.reshape(L // 8, 8, 128)

    def tile_rows(ref):
        return _unwords(ref[...].reshape(L * 8, 128))

    def emit(groups, o1, o2):
        for n, g in enumerate(groups):
            a, b = o1[:, 128 * n:128 * (n + 1)], o2[:, 128 * n:128 * (n + 1)]
            dst = v_s if g >= NG else k_s
            t = g % NG
            if t < 24:
                put(dst[t // 8], t % 8, _pack2(a, b))
                continue
            for i, v in enumerate((a, b)):
                w = _pack2(v, v) & half_mask
                if g >= NG:
                    w = w | pltpu.roll(w, 64, 1)
                put(dst[3], 2 * (t - 24) + i, w)

    def weights(ref, groups, rows=slice(None)):
        return jnp.concatenate([_unwords(ref[g, rows, :]) for g in groups], axis=1)

    def project(groups, lhs1, lhs2, lhsc):
        c = _dot(lhsc, weights(wc_s, groups))
        emit(groups, _dot(lhs1, weights(w1_s, groups)) + c, _dot(lhs2, weights(w2_s, groups)) + c)

    def project_by_tile(groups, lhs1, lhs2, lhsc):
        o1 = o2 = _dot(lhsc, weights(wc_s, groups))
        for k in range(3):
            rows, cols = slice(64 * k, 64 * (k + 1)), slice(128 * k, 128 * (k + 1))
            o1 = o1 + _dot(lhs1[:, cols], weights(w1_s, groups, rows))
            o2 = o2 + _dot(lhs2[:, cols], weights(w2_s, groups, rows))
        emit(groups, o1, o2)

    def over_keys(v, op):
        for d in (2, 4, 8):
            v = op(v, jnp.where((lane & d) == 0, pltpu.roll(v, 128 - d, 1), pltpu.roll(v, d, 1)))
        return v

    def step(b, i, carry):
        mem, best = carry
        z = jnp.concatenate([_unwords(y_s[n_blk, seg_rows(0), :]).astype(F32), mem], axis=0)
        if i:
            best = finish_segment(b, i - 1, None, best)
        else:
            best = finish_segment(jnp.maximum(b - 1, 0), BLK // SEG - 1,
                                  jnp.broadcast_to(b, (SEG, 1)) > 0, best)
        if i + 1 < BLK // SEG:
            norm_segment(b, i + 1)
        else:
            norm_segment(jnp.minimum(b + 1, n_blk - 1), 0)

        z0, z7 = z[:, 0:128], z[:, 384:512]
        lhs = (z[:, 0:384],
               jnp.concatenate([jnp.where(left, z7, z0), z[:, 128:384]], axis=1),
               jnp.where(left, z0, z7))
        order = list(range(24, NG)) + list(range(24))
        chunks = [order[n:n + CHUNK] for n in range(0, NG, CHUNK)]
        completes = {NG - 1: 3, 7: 0, 15: 1, 23: 2}
        keys = {}
        for n, groups in enumerate(chunks):
            (project if n else project_by_tile)(groups, *lhs)
            if groups[-1] in completes:
                j = completes[groups[-1]]
                keys[j] = tile_rows(k_s[j]).T
        chunks = [[NG + g for g in groups] for groups in chunks]
        for groups in chunks[:LEAD // CHUNK]:
            project(groups, *lhs)

        scores = []
        for n in range(L // 8):
            q0 = 8 * n if 8 * n < SEG else 0
            t = _dot(z[q0:L], jnp.concatenate(
                [keys[j][:, 128 * n:128 * (n + 1)] for j in range(4)], axis=0))
            if 8 * n < SEG:
                t = jnp.concatenate([jnp.where(causal, t[0:8], MASKED), t[8:]], axis=0)
            if q0:
                t = jnp.concatenate([jnp.full((q0, 128), MASKED, F32), t], axis=0)
            scores.append(t)
        top = over_keys(functools.reduce(jnp.maximum, scores), jnp.maximum)
        ex = [jnp.exp(t - top) for t in scores]
        inv = 1.0 / over_keys(functools.reduce(jnp.add, ex), jnp.add)
        p = _r16(jnp.concatenate([e * inv for e in ex], axis=1))
        for groups in chunks[LEAD // CHUNK:]:
            project(groups, *lhs)

        o = _dot(p, jnp.concatenate([tile_rows(v_s[j]) for j in (3, 0, 1, 2)], axis=1))
        o = _r16(jnp.concatenate([o[:, 128:512], o[:, 0:128]], axis=1))
        o_s[...] = o[0:SEG]
        return o[SEG:L], best

    def block(b, carry):
        for i in range(BLK // SEG):
            carry = step(b, i, carry)
        load_tokens(jnp.minimum(b + 2, n_blk - 1))
        store_tokens(jnp.maximum(b - 1, 0))

        @pl.when(b > 0)
        def _():
            out_copy(b - 1).start()
        return carry

    mem = _repeat_tail(mem0_v[...].astype(F32), 1)
    best = (jnp.full((SEG, 1), -jnp.inf, F32), lax.broadcasted_iota(jnp.int32, (SEG, 1), 0))
    _, best = lax.fori_loop(0, n_blk, block, (mem, best))
    arrive(cp_ffn)
    best_r, best_i = finish_segment(n_blk - 1, BLK // SEG - 1, None, best)
    store_tokens(n_blk - 1)

    idx = jnp.min(jnp.where(best_r == jnp.max(best_r), best_i, n_blk * BLK - 1))
    sel_b = idx // BLK
    sel_rows = pl.ds(pl.multiple_of(((idx - sel_b * BLK) // 16) * 8, 8), 8)
    x1 = _unwords(x1_s[sel_b, sel_rows, :]).astype(F32)
    h2 = _ln_mod(x1, vec(CB, 16), vec(SB, 16)).astype(F32)
    r = _r16(_row_sum(h2 * vec(WR, 16)))
    g = _r16(_dot(h2[:, 0:D], wg_v[...]))
    u = _r16(_dot(h2[:, 0:D], wu_v[...]))
    out_copy(n_blk - 1).start()
    g = _r16(g * jax.nn.sigmoid(g))
    y = _r16(_dot_nt(_r16(g * u), _repeat_tail(wd_v[...], 0)))
    y = _r16(y * _r16(jax.nn.sigmoid(r)))
    hit = lax.broadcasted_iota(jnp.int32, (16, 1), 0) == idx % 16
    upd = h2 * 0.0 + jnp.where(hit, y, 0.0)
    y_s[sel_b, sel_rows, :] = _words(x1 + vec(GB, 16) * _r16(h2 + upd))
    for b in range(n_blk):
        out_copy(b).wait()
    store_tokens(sel_b)
    last = out_copy(sel_b)
    last.start()
    last.wait()


@jax.jit
def pallas_adaLN_cond__memory_aug_recurrent_mem_tr__moe_arch_mod__prompt_kernel(
    A_x: jax.Array,
    A_mem0: jax.Array,
    A_Wq: jax.Array,
    A_Wk: jax.Array,
    A_Wv: jax.Array,
    A_Wo: jax.Array,
    A_seg_len: jax.Array,
    B_x: jax.Array,
    B_w_r: jax.Array,
    B_w_gate: jax.Array,
    B_w_up: jax.Array,
    B_w_down: jax.Array,
    c: jax.Array,
    w_mod: jax.Array,
):
    del A_seg_len, B_x
    _, S, _ = A_x.shape
    F = B_w_gate.shape[1]
    assert A_x.shape == (1, S, D) and S % BLK == 0
    assert A_mem0.shape == (1, M, D) and A_Wq.shape == (D, H, DH)
    n_blk = S // BLK
    hbm = pl.BlockSpec(memory_space=pltpu.HBM)
    head_words = pltpu.VMEM((2, D * H // 2 + 8, 128), U32)
    token_words = pltpu.VMEM((n_blk, BLK // 2, DP), U32)
    block_words = pltpu.VMEM((n_blk, D // 2, BLK), U32)
    out_t = pl.pallas_call(
        functools.partial(_kernel, n_blk=n_blk),
        out_shape=jax.ShapeDtypeStruct((D, S), BF16),
        in_specs=[hbm] * 12,
        out_specs=hbm,
        scratch_shapes=[
            pltpu.VMEM((1, D), BF16),
            pltpu.VMEM((M, D), BF16),
            pltpu.VMEM((D,), BF16),
            block_words,
            head_words, head_words, head_words,
            pltpu.VMEM((H * D, DH), BF16),
            pltpu.VMEM((D, F), BF16),
            pltpu.VMEM((D, F), BF16),
            pltpu.VMEM((D, F), BF16),
            pltpu.VMEM((D, 6 * D), BF16),
            pltpu.VMEM((H, D // 2, DH), U32),
            pltpu.VMEM((2 * NG, 192, 128), U32),
            pltpu.VMEM((2 * NG, 192, 128), U32),
            pltpu.VMEM((2 * NG, 64, 128), U32),
            *[pltpu.VMEM((L // 8, 64, 128), U32)] * 8,
            token_words,
            pltpu.VMEM((SEG, DP), F32),
            token_words,
            pltpu.VMEM((n_blk + 1, BLK // 2, DP), U32),
            block_words,
            pltpu.VMEM((7, 8, DP), F32),
            pltpu.SemaphoreType.DMA((23 + n_blk,)),
            pltpu.SemaphoreType.DMA(()),
        ],
        compiler_params=pltpu.CompilerParams(vmem_limit_bytes=100 * 1024 * 1024),
    )(A_x.reshape(S, D).T, A_mem0.reshape(M, D), A_Wq.reshape(D * H, DH),
      A_Wk.reshape(D * H, DH), A_Wv.reshape(D * H, DH),
      A_Wo.transpose(0, 2, 1).reshape(H * D, DH),
      B_w_r, B_w_gate, B_w_up, B_w_down.T, c, w_mod)
    return out_t.T.reshape(A_x.shape)
```

```python
import functools

import jax
import jax.numpy as jnp
from jax import lax
import jax.experimental.pallas as pl
import jax.experimental.pallas.tpu as pltpu

F32 = jnp.float32
BF16 = jnp.bfloat16
U32 = jnp.uint32

D = 448
DP = 512
H = 16
DH = 256
M = 8
SEG = 32
L = SEG + M
BLK = 128
NT = L // 8
NG = 28
EPS = 1e-5
MASKED = -1e9

HALVES = ((0, D // 2), (D // 2, D))
K_CHUNKS = ((0, 128), (128, D))
AHEAD = 3
CHUNK = 4
LEAD = 8


def _r16(x):
    return x.astype(BF16).astype(F32)


def _dot(a, b):
    return lax.dot_general(a, b, (((1,), (0,)), ((), ())), preferred_element_type=F32)


def _dot_nt(a, b):
    return lax.dot_general(a, b, (((1,), (1,)), ((), ())), preferred_element_type=F32)


def _words(x):
    return pltpu.bitcast(x.astype(BF16), U32)


def _unwords(w):
    return pltpu.bitcast(w, BF16)


def _pack2(a, b):
    return (pltpu.bitcast(_r16(a), U32) >> 16) | pltpu.bitcast(_r16(b), U32)


def _repeat_tail(x, axis):
    return jnp.concatenate([x, lax.slice_in_dim(x, D - 64, D, axis=axis)], axis=axis)


def _row_sum(x):
    left = lax.broadcasted_iota(jnp.int32, (x.shape[0], 128), 1) < 64
    t = (x[:, 0:128] + x[:, 128:256]) + (x[:, 256:384] + jnp.where(left, x[:, 384:512], 0.0))
    return jnp.sum(t, axis=1, keepdims=True)


def _ln_mod(x, scale1, shift):
    xc = x - _row_sum(x) / D
    var = _row_sum(xc * xc) / D
    den = _r16(jnp.sqrt(_r16(_r16(var) + _r16(jnp.float32(EPS)))))
    return ((xc / den) * scale1 + shift).astype(BF16)


def _kernel(x_hbm, mem0_hbm, wq_hbm, wk_hbm, wv_hbm, wo_hbm, wr_hbm, wg_hbm, wu_hbm, wd_hbm,
            c_hbm, wmod_hbm, out_hbm,
            c_v, mem0_v, wr_v, x_v, wq_v, wk_v, wv_v, wo_v, wg_v, wu_v, wd_v, wmod_v,
            qh_s, w1_s, w2_s, wc_s, k0_s, k1_s, k2_s, k3_s, v0_s, v1_s, v2_s, v3_s,
            xs_s, h_s, o_s, x1_s, out_v, vec_s, sems, out_sem, *, n_blk):
    k_s = (k0_s, k1_s, k2_s, k3_s)
    v_s = (v0_s, v1_s, v2_s, v3_s)

    def put_y(b, rows, words):
        for j in range(4):
            k0_s[NT + 4 * b + j, rows, :] = words[:, 128 * j:128 * (j + 1)]

    def get_y(b):
        return jnp.concatenate([k0_s[NT + 4 * b + j] for j in range(4)], axis=1)

    queue = []
    issued = [0]

    def fetch(src, dst):
        queue.append(pltpu.make_async_copy(src, dst, sems.at[len(queue)]))
        return len(queue) - 1

    def fetch_rows(src, dst, r0, r1):
        return [fetch(src.at[pl.ds(r0 * H, (r1 - r0) * H), pl.ds(128 * j, 128)],
                      dst.at[j, pl.ds(r0 * H // 2, (r1 - r0) * H // 2), :].bitcast(BF16))
                for j in range(2)]

    def issue(upto):
        while issued[0] < min(upto, len(queue)):
            queue[issued[0]].start()
            issued[0] += 1

    def arrive(copies):
        for i in copies:
            issue(i + AHEAD + 1)
            queue[i].wait()

    cp_q = [fetch_rows(wq_hbm, wq_v, r0, r1) for r0, r1 in HALVES]
    cp_k = [fetch_rows(wk_hbm, wk_v, r0, r1) for r0, r1 in K_CHUNKS]
    cp_v = [fetch_rows(wv_hbm, wv_v, r0, r1) for r0, r1 in HALVES]
    cp_o = [fetch(wo_hbm.at[pl.ds(4 * D * t, 4 * D), :], wo_v.at[pl.ds(4 * D * t, 4 * D), :])
            for t in range(H // 4)]
    cp_small = [fetch(c_hbm, c_v), fetch(mem0_hbm, mem0_v), fetch(wr_hbm, wr_v),
                fetch(wmod_hbm, wmod_v)]
    cp_x = [fetch(x_hbm.at[:, pl.ds(BLK * b, BLK)], x_v.at[b].bitcast(BF16))
            for b in range(n_blk)]
    cp_ffn = [fetch(wg_hbm, wg_v), fetch(wu_hbm, wu_v), fetch(wd_hbm, wd_v)]

    def head_pair(w_v, s, r0, r1):
        words = jnp.concatenate(
            [w_v[j, pl.ds(r0 * 8 + s, r1 - r0, stride=8), :] for j in range(2)], axis=1)
        return (pltpu.bitcast(words << 16, F32),
                pltpu.bitcast(words & jnp.uint32(0xFFFF0000), F32))

    def store_group(g, xw, yw, r0, r1):
        if r0 == 0:
            y1 = _r16(yw[0:64])
            w1_s[g, 0:32, :] = _words(xw[0:64] - y1)
            wc_s[g, 0:32, :] = _words(y1)
        lo, hi = max(r0, 64), min(r1, 384)
        w1_s[g, lo // 2:hi // 2, :] = _words(xw[lo - r0:hi - r0])
        w2_s[g, lo // 2:hi // 2, :] = _words(yw[lo - r0:hi - r0])
        if r1 == D:
            x7 = _r16(xw[384 - r0:])
            w2_s[g, 0:32, :] = _words(yw[384 - r0:] - x7)
            wc_s[g, 32:64, :] = _words(x7)

    def fold(base, lhs_v, rhs_pair, scale, r0, r1, unroll, before=None):
        def body(t, carry):
            if before is not None:
                before(t)
            tails = []
            for i in range(2):
                s = 2 * t + i
                la, lb = head_pair(lhs_v, s, r0, r1)
                ra, rb = rhs_pair(s)
                pa = _dot_nt(la, ra[0:384])
                pad = -(r1 - r0) % 128
                parts = []
                for lhs, rhs in ((la, ra), (lb, rb)):
                    lhs = lhs.astype(BF16)
                    if pad:
                        lhs = jnp.concatenate([lhs, lhs[0:pad]], axis=0)
                    parts.append(_dot_nt(rhs[384:D], lhs))
                tail = jnp.concatenate(parts, axis=0).T[0:r1 - r0]
                pb = _dot_nt(lb, rb[0:384])
                if scale is not None:
                    pa, pb, tail = pa * scale, pb * scale, tail * scale
                tails.append(tail)
                if i:
                    store_group(base + 24 + t, tails[0], tails[1], r0, r1)
                for j in range(3):
                    store_group(base + 8 * j + s, pa[:, 128 * j:128 * (j + 1)],
                                pb[:, 128 * j:128 * (j + 1)], r0, r1)
            return carry
        lax.fori_loop(0, H // 4, body, 0, unroll=unroll)

    def split_q_heads(r0, r1):
        def body(s, carry):
            for i, q in enumerate(head_pair(wq_v, s, r0, r1)):
                qh_s[2 * s + i, r0 // 2:r1 // 2, :] = _words(q)
            return carry
        lax.fori_loop(0, H // 2, body, 0)

    def q_pair(s):
        return _unwords(qh_s[2 * s]), _unwords(qh_s[2 * s + 1])

    def o_pair(s):
        r0 = pl.multiple_of(s * 2 * D, 2 * D)
        return wo_v[pl.ds(r0, D), :], wo_v[pl.ds(r0 + D, D), :]

    def o_arrive(t):
        rows = pl.ds(pl.multiple_of(t * 4 * D, 4 * D), 4 * D)
        pltpu.make_async_copy(wo_hbm.at[rows, :], wo_v.at[rows, :], sems.at[cp_o[0] + t]).wait()

    for copies, (r0, r1) in zip(cp_q, HALVES):
        arrive(copies)
        split_q_heads(r0, r1)
    for copies, (r0, r1) in zip(cp_k, K_CHUNKS):
        arrive(copies)
        if r1 == D:
            issue(cp_o[-1] + 1)
        fold(0, wk_v, q_pair, DH ** -0.5, r0, r1, 4 if r0 else 2)
    for copies in cp_v:
        arrive(copies)
    issue(len(queue))
    fold(NG, wv_v, o_pair, None, 0, D, 2, o_arrive)

    SA, CA, GA, SB, CB, GB, WR = range(7)

    def vec(i, rows):
        return jnp.concatenate([vec_s[i]] * (rows // 8), axis=0)

    def seg_rows(i):
        return slice(SEG // 2 * i, SEG // 2 * (i + 1))

    def load_tokens(b):
        xs_s[b] = pltpu.bitcast(_repeat_tail(_unwords(x_v[b]), 0).T, U32)

    def store_tokens(b):
        out_v[b] = pltpu.bitcast(_unwords(get_y(b)).T[0:D], U32)

    def out_copy(b):
        lanes = pl.ds(pl.multiple_of(b * BLK, BLK), BLK)
        return pltpu.make_async_copy(out_v.at[b].bitcast(BF16), out_hbm.at[:, lanes], out_sem)

    def norm_segment(b, i):
        x = _unwords(xs_s[b, seg_rows(i), :]).astype(F32)
        h_s[...] = pltpu.bitcast(_ln_mod(x, vec(CA, SEG), vec(SA, SEG)), U32)

    def finish_segment(b, i, valid, best):
        x1 = (_unwords(xs_s[b, seg_rows(i), :]).astype(F32)
              + _r16(vec(GA, SEG) * o_s[...])).astype(BF16)
        x1_s[b, seg_rows(i), :] = pltpu.bitcast(x1, U32)
        x1 = x1.astype(F32)
        h2 = _ln_mod(x1, vec(CB, SEG), vec(SB, SEG)).astype(F32)
        r = _r16(_row_sum(h2 * vec(WR, SEG)))
        put_y(b, seg_rows(i), _words(x1 + vec(GB, SEG) * (h2 + h2 * 0.0)))
        better = r > best[0]
        if valid is not None:
            better = better & valid
        idx = b * BLK + SEG * i + lax.broadcasted_iota(jnp.int32, (SEG, 1), 0)
        return jnp.where(better, r, best[0]), jnp.where(better, idx, best[1])

    arrive(cp_small + cp_x)
    load_tokens(0)
    load_tokens(min(1, n_blk - 1))
    cf = jnp.broadcast_to(c_v[...].astype(F32), (8, D))
    mod = _r16(_dot(_r16(cf * jax.nn.sigmoid(cf)), wmod_v[...]))
    for i in range(6):
        v = mod[:, D * i:D * (i + 1)]
        vec_s[i] = _repeat_tail(_r16(1.0 + v) if i in (CA, CB) else v, 1)
    vec_s[WR] = _repeat_tail(jnp.broadcast_to(wr_v[...].astype(F32).reshape(1, D), (8, D)), 1)
    norm_segment(0, 0)
    o_s[...] = jnp.zeros(o_s.shape, F32)

    lane = lax.broadcasted_iota(jnp.int32, (L, 128), 1)
    left = lane < 64
    half_mask = jnp.where(left, jnp.uint32(0x0000FFFF), jnp.uint32(0xFFFF0000))
    causal = ((lax.broadcasted_iota(jnp.int32, (8, 128), 1) % 16) // 2
              <= lax.broadcasted_iota(jnp.int32, (8, 128), 0))

    def put(ref, s, words):
        ref[0:NT, 8 * s:8 * (s + 1), :] = words.reshape(NT, 8, 128)

    def tile_rows(ref):
        return _unwords(ref[0:NT].reshape(L * 8, 128))

    def emit(groups, o1, o2):
        for n, g in enumerate(groups):
            a, b = o1[:, 128 * n:128 * (n + 1)], o2[:, 128 * n:128 * (n + 1)]
            dst = v_s if g >= NG else k_s
            t = g % NG
            if t < 24:
                put(dst[t // 8], t % 8, _pack2(a, b))
                continue
            for i, v in enumerate((a, b)):
                w = _pack2(v, v) & half_mask
                if g >= NG:
                    w = w | pltpu.roll(w, 64, 1)
                put(dst[3], 2 * (t - 24) + i, w)

    def weights(ref, groups, rows=slice(None)):
        return jnp.concatenate([_unwords(ref[g, rows, :]) for g in groups], axis=1)

    def project(groups, lhs1, lhs2, lhsc):
        c = _dot(lhsc, weights(wc_s, groups))
        emit(groups, _dot(lhs1, weights(w1_s, groups)) + c, _dot(lhs2, weights(w2_s, groups)) + c)

    def project_by_tile(groups, lhs1, lhs2, lhsc):
        o1 = o2 = _dot(lhsc, weights(wc_s, groups))
        for k in range(3):
            rows, cols = slice(64 * k, 64 * (k + 1)), slice(128 * k, 128 * (k + 1))
            o1 = o1 + _dot(lhs1[:, cols], weights(w1_s, groups, rows))
            o2 = o2 + _dot(lhs2[:, cols], weights(w2_s, groups, rows))
        emit(groups, o1, o2)

    def over_keys(v, op):
        for d in (2, 4, 8):
            v = op(v, jnp.where((lane & d) == 0, pltpu.roll(v, 128 - d, 1), pltpu.roll(v, d, 1)))
        return v

    def step(b, i, carry):
        mem, best = carry
        z = jnp.concatenate([_unwords(h_s[...]).astype(F32), mem], axis=0)
        if i:
            best = finish_segment(b, i - 1, None, best)
        else:
            best = finish_segment(jnp.maximum(b - 1, 0), BLK // SEG - 1,
                                  jnp.broadcast_to(b, (SEG, 1)) > 0, best)
        if i + 1 < BLK // SEG:
            norm_segment(b, i + 1)
        else:
            norm_segment(jnp.minimum(b + 1, n_blk - 1), 0)

        z0, z7 = z[:, 0:128], z[:, 384:512]
        lhs = (z[:, 0:384],
               jnp.concatenate([jnp.where(left, z7, z0), z[:, 128:384]], axis=1),
               jnp.where(left, z0, z7))
        order = list(range(24, NG)) + list(range(24))
        chunks = [order[n:n + CHUNK] for n in range(0, NG, CHUNK)]
        completes = {NG - 1: 3, 7: 0, 15: 1, 23: 2}
        keys = {}
        for n, groups in enumerate(chunks):
            (project if n else project_by_tile)(groups, *lhs)
            if groups[-1] in completes:
                j = completes[groups[-1]]
                keys[j] = tile_rows(k_s[j]).T
        chunks = [[NG + g for g in groups] for groups in chunks]
        for groups in chunks[:LEAD // CHUNK]:
            project(groups, *lhs)

        scores = [None] * NT
        for n in (0, 3, 4, 2, 1):
            q0 = 8 * n if 8 * n < SEG else 0
            t = _dot(z[q0:L], jnp.concatenate(
                [keys[j][:, 128 * n:128 * (n + 1)] for j in range(4)], axis=0))
            if 8 * n < SEG:
                t = jnp.concatenate([jnp.where(causal, t[0:8], MASKED), t[8:]], axis=0)
            if q0:
                t = jnp.concatenate([jnp.full((q0, 128), MASKED, F32), t], axis=0)
            scores[n] = t
        top = over_keys(functools.reduce(jnp.maximum, scores), jnp.maximum)
        ex = [jnp.exp(t - top) for t in scores]
        inv = 1.0 / over_keys(functools.reduce(jnp.add, ex), jnp.add)
        p = _r16(jnp.concatenate([e * inv for e in ex], axis=1))
        for groups in chunks[LEAD // CHUNK:]:
            project(groups, *lhs)

        o = _dot(p, jnp.concatenate([tile_rows(v_s[j]) for j in (3, 0, 1, 2)], axis=1))
        o = _r16(jnp.concatenate([o[:, 128:512], o[:, 0:128]], axis=1))
        o_s[...] = o[0:SEG]
        return o[SEG:L], best

    def block(b, carry):
        for i in range(BLK // SEG):
            carry = step(b, i, carry)
        load_tokens(jnp.minimum(b + 2, n_blk - 1))
        store_tokens(jnp.maximum(b - 1, 0))

        @pl.when(b > 0)
        def _():
            out_copy(b - 1).start()
        return carry

    mem = _repeat_tail(mem0_v[...].astype(F32), 1)
    best = (jnp.full((SEG, 1), -jnp.inf, F32), lax.broadcasted_iota(jnp.int32, (SEG, 1), 0))
    _, best = lax.fori_loop(0, n_blk, block, (mem, best))
    arrive(cp_ffn)
    best_r, best_i = finish_segment(n_blk - 1, BLK // SEG - 1, None, best)
    store_tokens(n_blk - 1)

    idx = jnp.min(jnp.where(best_r == jnp.max(best_r), best_i, n_blk * BLK - 1))
    sel_b = idx // BLK
    sel_rows = pl.ds(pl.multiple_of(((idx - sel_b * BLK) // 16) * 8, 8), 8)
    x1 = _unwords(x1_s[sel_b, sel_rows, :]).astype(F32)
    h2 = _ln_mod(x1, vec(CB, 16), vec(SB, 16)).astype(F32)
    r = _r16(_row_sum(h2 * vec(WR, 16)))
    g = _r16(_dot(h2[:, 0:D], wg_v[...]))
    u = _r16(_dot(h2[:, 0:D], wu_v[...]))
    out_copy(n_blk - 1).start()
    g = _r16(g * jax.nn.sigmoid(g))
    y = _r16(_dot_nt(_r16(g * u), _repeat_tail(wd_v[...], 0)))
    y = _r16(y * _r16(jax.nn.sigmoid(r)))
    hit = lax.broadcasted_iota(jnp.int32, (16, 1), 0) == idx % 16
    upd = h2 * 0.0 + jnp.where(hit, y, 0.0)
    put_y(sel_b, sel_rows, _words(x1 + vec(GB, 16) * _r16(h2 + upd)))
    for b in range(n_blk):
        out_copy(b).wait()
    store_tokens(sel_b)
    last = out_copy(sel_b)
    last.start()
    last.wait()


@jax.jit
def pallas_adaLN_cond__memory_aug_recurrent_mem_tr__moe_arch_mod__prompt_kernel(
    A_x: jax.Array,
    A_mem0: jax.Array,
    A_Wq: jax.Array,
    A_Wk: jax.Array,
    A_Wv: jax.Array,
    A_Wo: jax.Array,
    A_seg_len: jax.Array,
    B_x: jax.Array,
    B_w_r: jax.Array,
    B_w_gate: jax.Array,
    B_w_up: jax.Array,
    B_w_down: jax.Array,
    c: jax.Array,
    w_mod: jax.Array,
):
    del A_seg_len, B_x
    _, S, _ = A_x.shape
    F = B_w_gate.shape[1]
    assert A_x.shape == (1, S, D) and S % BLK == 0
    assert A_mem0.shape == (1, M, D) and A_Wq.shape == (D, H, DH)
    n_blk = S // BLK
    hbm = pl.BlockSpec(memory_space=pltpu.HBM)
    head_words = pltpu.VMEM((2, D * H // 2 + 8, 128), U32)
    token_words = pltpu.VMEM((n_blk, BLK // 2, DP), U32)
    block_words = pltpu.VMEM((n_blk, D // 2, BLK), U32)
    out_t = pl.pallas_call(
        functools.partial(_kernel, n_blk=n_blk),
        out_shape=jax.ShapeDtypeStruct((D, S), BF16),
        in_specs=[hbm] * 12,
        out_specs=hbm,
        scratch_shapes=[
            pltpu.VMEM((1, D), BF16),
            pltpu.VMEM((M, D), BF16),
            pltpu.VMEM((D,), BF16),
            block_words,
            head_words, head_words, head_words,
            pltpu.VMEM((H * D, DH), BF16),
            pltpu.VMEM((D, F), BF16),
            pltpu.VMEM((D, F), BF16),
            pltpu.VMEM((D, F), BF16),
            pltpu.VMEM((D, 6 * D), BF16),
            pltpu.VMEM((H, D // 2, DH), U32),
            pltpu.VMEM((2 * NG, 192, 128), U32),
            pltpu.VMEM((2 * NG, 192, 128), U32),
            pltpu.VMEM((2 * NG, 64, 128), U32),
            pltpu.VMEM((NT + 4 * n_blk, 64, 128), U32),
            *[pltpu.VMEM((NT, 64, 128), U32)] * 7,
            token_words,
            pltpu.VMEM((SEG // 2, DP), U32),
            pltpu.VMEM((SEG, DP), F32),
            token_words,
            block_words,
            pltpu.VMEM((7, 8, DP), F32),
            pltpu.SemaphoreType.DMA((23 + n_blk,)),
            pltpu.SemaphoreType.DMA(()),
        ],
        compiler_params=pltpu.CompilerParams(vmem_limit_bytes=100 * 1024 * 1024),
    )(A_x.reshape(S, D).T, A_mem0.reshape(M, D), A_Wq.reshape(D * H, DH),
      A_Wk.reshape(D * H, DH), A_Wv.reshape(D * H, DH),
      A_Wo.transpose(0, 2, 1).reshape(H * D, DH),
      B_w_r, B_w_gate, B_w_up, B_w_down.T, c, w_mod)
    return out_t.T.reshape(A_x.shape)
```

```python
import functools

import jax
import jax.numpy as jnp
import numpy as np
from jax import lax
import jax.experimental.pallas as pl
import jax.experimental.pallas.tpu as pltpu

F32 = jnp.float32
BF16 = jnp.bfloat16
U32 = jnp.uint32

D = 448
DP = 512
H = 16
DH = 256
M = 8
SEG = 32
L = SEG + M
BLK = 128
NT = L // 8
NG = 28
EPS = float(np.asarray(1e-5, dtype=BF16))
MASKED = -1e9

HALVES = ((0, D // 2), (D // 2, D))
K_CHUNKS = ((0, 128), (128, D))
AHEAD = 3
CHUNK = 4
LEAD = 8


def _r16(x):
    return x.astype(BF16).astype(F32)


def _dot(a, b):
    return lax.dot_general(a, b, (((1,), (0,)), ((), ())), preferred_element_type=F32)


def _dot_nt(a, b):
    return lax.dot_general(a, b, (((1,), (1,)), ((), ())), preferred_element_type=F32)


def _words(x):
    return pltpu.bitcast(x.astype(BF16), U32)


def _unwords(w):
    return pltpu.bitcast(w, BF16)


def _pack2(a, b):
    return (pltpu.bitcast(_r16(a), U32) >> 16) | pltpu.bitcast(_r16(b), U32)


def _repeat_tail(x, axis):
    return jnp.concatenate([x, lax.slice_in_dim(x, D - 64, D, axis=axis)], axis=axis)


def _row_sum(x):
    left = lax.broadcasted_iota(jnp.int32, (x.shape[0], 128), 1) < 64
    t = (x[:, 0:128] + x[:, 128:256]) + (x[:, 256:384] + jnp.where(left, x[:, 384:512], 0.0))
    return jnp.sum(t, axis=1, keepdims=True)


def _ln_mod(x, scale1, shift):
    xc = x - _row_sum(x) / D
    var = _row_sum(xc * xc) / D
    den = _r16(jnp.sqrt(_r16(_r16(var) + EPS)))
    return ((xc / den) * scale1 + shift).astype(BF16)


def _kernel(x_hbm, mem0_hbm, wq_hbm, wk_hbm, wv_hbm, wo_hbm, wr_hbm, wg_hbm, wu_hbm, wd_hbm,
            c_hbm, wmod_hbm, out_hbm,
            c_v, mem0_v, wr_v, x_v, wq_v, wk_v, wv_v, wo_v, wg_v, wu_v, wd_v, wmod_v,
            qh_s, w1_s, w2_s, wc_s, k0_s, k1_s, k2_s, k3_s, v0_s, v1_s, v2_s, v3_s,
            xs_s, h_s, o_s, x1_s, out_v, vec_s, sems, out_sem, *, n_blk):
    k_s = (k0_s, k1_s, k2_s, k3_s)
    v_s = (v0_s, v1_s, v2_s, v3_s)

    def put_y(b, rows, words):
        for j in range(4):
            k0_s[NT + 4 * b + j, rows, :] = words[:, 128 * j:128 * (j + 1)]

    def get_y(b):
        return jnp.concatenate([k0_s[NT + 4 * b + j] for j in range(4)], axis=1)

    queue = []
    issued = [0]

    def fetch(src, dst):
        queue.append(pltpu.make_async_copy(src, dst, sems.at[len(queue)]))
        return len(queue) - 1

    def fetch_rows(src, dst, r0, r1):
        return [fetch(src.at[pl.ds(r0 * H, (r1 - r0) * H), pl.ds(128 * j, 128)],
                      dst.at[j, pl.ds(r0 * H // 2, (r1 - r0) * H // 2), :].bitcast(BF16))
                for j in range(2)]

    def issue(upto):
        while issued[0] < min(upto, len(queue)):
            queue[issued[0]].start()
            issued[0] += 1

    def arrive(copies):
        for i in copies:
            issue(i + AHEAD + 1)
            queue[i].wait()

    cp_q = [fetch_rows(wq_hbm, wq_v, r0, r1) for r0, r1 in HALVES]
    cp_k = [fetch_rows(wk_hbm, wk_v, r0, r1) for r0, r1 in K_CHUNKS]
    cp_v = [fetch_rows(wv_hbm, wv_v, r0, r1) for r0, r1 in HALVES]
    cp_o = [fetch(wo_hbm.at[pl.ds(4 * D * t, 4 * D), :], wo_v.at[pl.ds(4 * D * t, 4 * D), :])
            for t in range(H // 4)]
    cp_small = [fetch(c_hbm, c_v), fetch(mem0_hbm, mem0_v), fetch(wr_hbm, wr_v),
                fetch(wmod_hbm, wmod_v)]
    cp_x = [fetch(x_hbm.at[:, pl.ds(BLK * b, BLK)], x_v.at[b].bitcast(BF16))
            for b in range(n_blk)]
    cp_ffn = [fetch(wg_hbm, wg_v), fetch(wu_hbm, wu_v), fetch(wd_hbm, wd_v)]

    def head_pair(w_v, s, r0, r1):
        words = jnp.concatenate(
            [w_v[j, pl.ds(r0 * 8 + s, r1 - r0, stride=8), :] for j in range(2)], axis=1)
        return (pltpu.bitcast(words << 16, F32),
                pltpu.bitcast(words & np.uint32(0xFFFF0000), F32))

    def store_group(g, xw, yw, r0, r1):
        if r0 == 0:
            y1 = _r16(yw[0:64])
            w1_s[g, 0:32, :] = _words(xw[0:64] - y1)
            wc_s[g, 0:32, :] = _words(y1)
        lo, hi = max(r0, 64), min(r1, 384)
        w1_s[g, lo // 2:hi // 2, :] = _words(xw[lo - r0:hi - r0])
        w2_s[g, lo // 2:hi // 2, :] = _words(yw[lo - r0:hi - r0])
        if r1 == D:
            x7 = _r16(xw[384 - r0:])
            w2_s[g, 0:32, :] = _words(yw[384 - r0:] - x7)
            wc_s[g, 32:64, :] = _words(x7)

    def fold(base, lhs_v, rhs_pair, scale, r0, r1, unroll, before=None):
        def body(t, carry):
            if before is not None:
                before(t)
            tails = []
            for i in range(2):
                s = 2 * t + i
                la, lb = head_pair(lhs_v, s, r0, r1)
                ra, rb = rhs_pair(s)
                pa = _dot_nt(la, ra[0:384])
                pad = -(r1 - r0) % 128
                parts = []
                for lhs, rhs in ((la, ra), (lb, rb)):
                    lhs = lhs.astype(BF16)
                    if pad:
                        lhs = jnp.concatenate([lhs, lhs[0:pad]], axis=0)
                    parts.append(_dot_nt(rhs[384:D], lhs))
                tail = jnp.concatenate(parts, axis=0).T[0:r1 - r0]
                pb = _dot_nt(lb, rb[0:384])
                if scale is not None:
                    pa, pb, tail = pa * scale, pb * scale, tail * scale
                tails.append(tail)
                if i:
                    store_group(base + 24 + t, tails[0], tails[1], r0, r1)
                for j in range(3):
                    store_group(base + 8 * j + s, pa[:, 128 * j:128 * (j + 1)],
                                pb[:, 128 * j:128 * (j + 1)], r0, r1)
            return carry
        lax.fori_loop(0, H // 4, body, 0, unroll=unroll)

    def split_q_heads(r0, r1):
        def body(s, carry):
            for i, q in enumerate(head_pair(wq_v, s, r0, r1)):
                qh_s[2 * s + i, r0 // 2:r1 // 2, :] = _words(q)
            return carry
        lax.fori_loop(0, H // 2, body, 0)

    def q_pair(s):
        return _unwords(qh_s[2 * s]), _unwords(qh_s[2 * s + 1])

    def o_pair(s):
        r0 = pl.multiple_of(s * 2 * D, 2 * D)
        return wo_v[pl.ds(r0, D), :], wo_v[pl.ds(r0 + D, D), :]

    def o_arrive(t):
        rows = pl.ds(pl.multiple_of(t * 4 * D, 4 * D), 4 * D)
        pltpu.make_async_copy(wo_hbm.at[rows, :], wo_v.at[rows, :], sems.at[cp_o[0] + t]).wait()

    for copies, (r0, r1) in zip(cp_q, HALVES):
        arrive(copies)
        split_q_heads(r0, r1)
    for copies, (r0, r1) in zip(cp_k, K_CHUNKS):
        arrive(copies)
        if r1 == D:
            issue(cp_o[-1] + 1)
        fold(0, wk_v, q_pair, DH ** -0.5, r0, r1, 4 if r0 else 2)
    for copies in cp_v:
        arrive(copies)
    issue(len(queue))
    fold(NG, wv_v, o_pair, None, 0, D, 2, o_arrive)

    SA, CA, GA, SB, CB, GB, WR = range(7)

    def vec(i, rows):
        return jnp.concatenate([vec_s[i]] * (rows // 8), axis=0)

    def seg_rows(i):
        return slice(SEG // 2 * i, SEG // 2 * (i + 1))

    def load_tokens(b):
        xs_s[b] = pltpu.bitcast(_repeat_tail(_unwords(x_v[b]), 0).T, U32)

    def store_tokens(b):
        out_v[b] = pltpu.bitcast(_unwords(get_y(b)).T[0:D], U32)

    def out_copy(b):
        lanes = pl.ds(pl.multiple_of(b * BLK, BLK), BLK)
        return pltpu.make_async_copy(out_v.at[b].bitcast(BF16), out_hbm.at[:, lanes], out_sem)

    def norm_segment(b, i):
        x = _unwords(xs_s[b, seg_rows(i), :]).astype(F32)
        h_s[...] = pltpu.bitcast(_ln_mod(x, vec(CA, SEG), vec(SA, SEG)), U32)

    def finish_segment(b, i, valid, best):
        x1 = (_unwords(xs_s[b, seg_rows(i), :]).astype(F32)
              + _r16(vec(GA, SEG) * o_s[...])).astype(BF16)
        x1_s[b, seg_rows(i), :] = pltpu.bitcast(x1, U32)
        x1 = x1.astype(F32)
        h2 = _ln_mod(x1, vec(CB, SEG), vec(SB, SEG)).astype(F32)
        r = _r16(_row_sum(h2 * vec(WR, SEG)))
        put_y(b, seg_rows(i), _words(x1 + vec(GB, SEG) * (h2 + h2 * 0.0)))
        better = r > best[0]
        if valid is not None:
            better = better & valid
        idx = b * BLK + SEG * i + lax.broadcasted_iota(jnp.int32, (SEG, 1), 0)
        return jnp.where(better, r, best[0]), jnp.where(better, idx, best[1])

    arrive(cp_small + cp_x)
    load_tokens(0)
    load_tokens(min(1, n_blk - 1))
    cf = jnp.broadcast_to(c_v[...].astype(F32), (8, D))
    mod = _r16(_dot(_r16(cf * jax.nn.sigmoid(cf)), wmod_v[...]))
    for i in range(6):
        v = mod[:, D * i:D * (i + 1)]
        vec_s[i] = _repeat_tail(_r16(1.0 + v) if i in (CA, CB) else v, 1)
    vec_s[WR] = _repeat_tail(jnp.broadcast_to(wr_v[...].astype(F32).reshape(1, D), (8, D)), 1)
    norm_segment(0, 0)
    o_s[...] = jnp.zeros(o_s.shape, F32)

    lane = lax.broadcasted_iota(jnp.int32, (L, 128), 1)
    left = lane < 64
    half_mask = jnp.where(left, np.uint32(0x0000FFFF), np.uint32(0xFFFF0000))
    causal = ((lax.broadcasted_iota(jnp.int32, (8, 128), 1) % 16) // 2
              <= lax.broadcasted_iota(jnp.int32, (8, 128), 0))

    def put(ref, s, words):
        ref[0:NT, 8 * s:8 * (s + 1), :] = words.reshape(NT, 8, 128)

    def tile_rows(ref):
        return _unwords(ref[0:NT].reshape(L * 8, 128))

    def emit(groups, o1, o2):
        for n, g in enumerate(groups):
            a, b = o1[:, 128 * n:128 * (n + 1)], o2[:, 128 * n:128 * (n + 1)]
            dst = v_s if g >= NG else k_s
            t = g % NG
            if t < 24:
                put(dst[t // 8], t % 8, _pack2(a, b))
                continue
            for i, v in enumerate((a, b)):
                w = _pack2(v, v) & half_mask
                if g >= NG:
                    w = w | pltpu.roll(w, 64, 1)
                put(dst[3], 2 * (t - 24) + i, w)

    def weights(ref, groups, rows=slice(None)):
        return jnp.concatenate([_unwords(ref[g, rows, :]) for g in groups], axis=1)

    def project(groups, lhs1, lhs2, lhsc):
        c = _dot(lhsc, weights(wc_s, groups))
        emit(groups, _dot(lhs1, weights(w1_s, groups)) + c, _dot(lhs2, weights(w2_s, groups)) + c)

    def project_by_tile(groups, lhs1, lhs2, lhsc):
        o1 = o2 = _dot(lhsc, weights(wc_s, groups))
        for k in range(3):
            rows, cols = slice(64 * k, 64 * (k + 1)), slice(128 * k, 128 * (k + 1))
            o1 = o1 + _dot(lhs1[:, cols], weights(w1_s, groups, rows))
            o2 = o2 + _dot(lhs2[:, cols], weights(w2_s, groups, rows))
        emit(groups, o1, o2)

    def over_keys(v, op):
        for d in (2, 4, 8):
            v = op(v, jnp.where((lane & d) == 0, pltpu.roll(v, 128 - d, 1), pltpu.roll(v, d, 1)))
        return v

    def step(b, i, carry):
        mem, best = carry
        z = jnp.concatenate([_unwords(h_s[...]).astype(F32), mem], axis=0)
        if i:
            best = finish_segment(b, i - 1, None, best)
        else:
            best = finish_segment(jnp.maximum(b - 1, 0), BLK // SEG - 1,
                                  jnp.broadcast_to(b, (SEG, 1)) > 0, best)
        if i + 1 < BLK // SEG:
            norm_segment(b, i + 1)
        else:
            norm_segment(jnp.minimum(b + 1, n_blk - 1), 0)

        z0, z7 = z[:, 0:128], z[:, 384:512]
        lhs = (z[:, 0:384],
               jnp.concatenate([jnp.where(left, z7, z0), z[:, 128:384]], axis=1),
               jnp.where(left, z0, z7))
        order = list(range(24, NG)) + list(range(24))
        chunks = [order[n:n + CHUNK] for n in range(0, NG, CHUNK)]
        completes = {NG - 1: 3, 7: 0, 15: 1, 23: 2}
        keys = {}
        for n, groups in enumerate(chunks):
            (project if n else project_by_tile)(groups, *lhs)
            if groups[-1] in completes:
                j = completes[groups[-1]]
                keys[j] = tile_rows(k_s[j]).T
        chunks = [[NG + g for g in groups] for groups in chunks]
        for groups in chunks[:LEAD // CHUNK]:
            project(groups, *lhs)

        scores = [None] * NT
        for n in (0, 3, 4, 2, 1):
            q0 = 8 * n if 8 * n < SEG else 0
            t = _dot(z[q0:L], jnp.concatenate(
                [keys[j][:, 128 * n:128 * (n + 1)] for j in range(4)], axis=0))
            if 8 * n < SEG:
                t = jnp.concatenate([jnp.where(causal, t[0:8], MASKED), t[8:]], axis=0)
            if q0:
                t = jnp.concatenate([jnp.full((q0, 128), MASKED, F32), t], axis=0)
            scores[n] = t
        top = over_keys(functools.reduce(jnp.maximum, scores), jnp.maximum)
        ex = [jnp.exp(t - top) for t in scores]
        inv = 1.0 / over_keys(functools.reduce(jnp.add, ex), jnp.add)
        p = _r16(jnp.concatenate([e * inv for e in ex], axis=1))
        for groups in chunks[LEAD // CHUNK:]:
            project(groups, *lhs)

        o = _dot(p, jnp.concatenate([tile_rows(v_s[j]) for j in (3, 0, 1, 2)], axis=1))
        o = _r16(jnp.concatenate([o[:, 128:512], o[:, 0:128]], axis=1))
        o_s[...] = o[0:SEG]
        return o[SEG:L], best

    def block(b, carry):
        for i in range(BLK // SEG):
            carry = step(b, i, carry)
        load_tokens(jnp.minimum(b + 2, n_blk - 1))
        store_tokens(jnp.maximum(b - 1, 0))

        @pl.when(b > 0)
        def _():
            out_copy(b - 1).start()
        return carry

    mem = _repeat_tail(mem0_v[...].astype(F32), 1)
    best = (jnp.full((SEG, 1), -jnp.inf, F32), lax.broadcasted_iota(jnp.int32, (SEG, 1), 0))
    _, best = lax.fori_loop(0, n_blk, block, (mem, best))
    arrive(cp_ffn)
    best_r, best_i = finish_segment(n_blk - 1, BLK // SEG - 1, None, best)
    store_tokens(n_blk - 1)

    idx = jnp.min(jnp.where(best_r == jnp.max(best_r), best_i, n_blk * BLK - 1))
    sel_b = idx // BLK
    sel_rows = pl.ds(pl.multiple_of(((idx - sel_b * BLK) // 16) * 8, 8), 8)
    x1 = _unwords(x1_s[sel_b, sel_rows, :]).astype(F32)
    h2 = _ln_mod(x1, vec(CB, 16), vec(SB, 16)).astype(F32)
    r = _r16(_row_sum(h2 * vec(WR, 16)))
    g = _r16(_dot(h2[:, 0:D], wg_v[...]))
    u = _r16(_dot(h2[:, 0:D], wu_v[...]))
    out_copy(n_blk - 1).start()
    g = _r16(g * jax.nn.sigmoid(g))
    y = _r16(_dot_nt(_r16(g * u), _repeat_tail(wd_v[...], 0)))
    y = _r16(y * _r16(jax.nn.sigmoid(r)))
    hit = lax.broadcasted_iota(jnp.int32, (16, 1), 0) == idx % 16
    upd = h2 * 0.0 + jnp.where(hit, y, 0.0)
    put_y(sel_b, sel_rows, _words(x1 + vec(GB, 16) * _r16(h2 + upd)))
    for b in range(n_blk):
        out_copy(b).wait()
    store_tokens(sel_b)
    last = out_copy(sel_b)
    last.start()
    last.wait()


@jax.jit
def pallas_adaLN_cond__memory_aug_recurrent_mem_tr__moe_arch_mod__prompt_kernel(
    A_x: jax.Array,
    A_mem0: jax.Array,
    A_Wq: jax.Array,
    A_Wk: jax.Array,
    A_Wv: jax.Array,
    A_Wo: jax.Array,
    A_seg_len: jax.Array,
    B_x: jax.Array,
    B_w_r: jax.Array,
    B_w_gate: jax.Array,
    B_w_up: jax.Array,
    B_w_down: jax.Array,
    c: jax.Array,
    w_mod: jax.Array,
):
    del A_seg_len, B_x
    _, S, _ = A_x.shape
    F = B_w_gate.shape[1]
    assert A_x.shape == (1, S, D) and S % BLK == 0
    assert A_mem0.shape == (1, M, D) and A_Wq.shape == (D, H, DH)
    n_blk = S // BLK
    hbm = pl.BlockSpec(memory_space=pltpu.HBM)
    head_words = pltpu.VMEM((2, D * H // 2 + 8, 128), U32)
    token_words = pltpu.VMEM((n_blk, BLK // 2, DP), U32)
    block_words = pltpu.VMEM((n_blk, D // 2, BLK), U32)
    out_t = pl.pallas_call(
        functools.partial(_kernel, n_blk=n_blk),
        out_shape=jax.ShapeDtypeStruct((D, S), BF16),
        in_specs=[hbm] * 12,
        out_specs=hbm,
        scratch_shapes=[
            pltpu.VMEM((1, D), BF16),
            pltpu.VMEM((M, D), BF16),
            pltpu.VMEM((D,), BF16),
            block_words,
            head_words, head_words, head_words,
            pltpu.VMEM((H * D, DH), BF16),
            pltpu.VMEM((D, F), BF16),
            pltpu.VMEM((D, F), BF16),
            pltpu.VMEM((D, F), BF16),
            pltpu.VMEM((D, 6 * D), BF16),
            pltpu.VMEM((H, D // 2, DH), U32),
            pltpu.VMEM((2 * NG, 192, 128), U32),
            pltpu.VMEM((2 * NG, 192, 128), U32),
            pltpu.VMEM((2 * NG, 64, 128), U32),
            pltpu.VMEM((NT + 4 * n_blk, 64, 128), U32),
            *[pltpu.VMEM((NT, 64, 128), U32)] * 7,
            token_words,
            pltpu.VMEM((SEG // 2, DP), U32),
            pltpu.VMEM((SEG, DP), F32),
            token_words,
            block_words,
            pltpu.VMEM((7, 8, DP), F32),
            pltpu.SemaphoreType.DMA((23 + n_blk,)),
            pltpu.SemaphoreType.DMA(()),
        ],
        compiler_params=pltpu.CompilerParams(vmem_limit_bytes=100 * 1024 * 1024),
    )(A_x.reshape(S, D).T, A_mem0.reshape(M, D), A_Wq.reshape(D * H, DH),
      A_Wk.reshape(D * H, DH), A_Wv.reshape(D * H, DH),
      A_Wo.transpose(0, 2, 1).reshape(H * D, DH),
      B_w_r, B_w_gate, B_w_up, B_w_down.T, c, w_mod)
    return out_t.T.reshape(A_x.shape)
```
